```python
import os as _os
_os.environ.setdefault("JAX_PLATFORMS", "cpu")
import jax
import jax.numpy as jnp

def _softmax(x, axis=-1):
    return jax.nn.softmax(x, axis=axis)
def _gelu(x):
    return jax.nn.gelu(x, approximate=True)
def _silu(x):
    return jax.nn.silu(x)
def _sigmoid(x):
    return jax.nn.sigmoid(x)
def _layernorm(x, axis=-1, eps=1e-5):
    m = jnp.mean(x, axis=axis, keepdims=True)
    v = jnp.var(x, axis=axis, keepdims=True)
    return (x - m) / jnp.sqrt(v + eps)
def _scatter_add(tgt, idx, src, axis=0):
    return tgt.at[idx].add(src)
def _segment_sum(src, seg, n):
    return jax.ops.segment_sum(src, seg, n)
class _Rng:
    def __init__(self, key):
        self._k = key
    def _next(self):
        self._k, sub = jax.random.split(self._k)
        return sub
    def normal(self, shape):
        return jax.random.normal(self._next(), shape, dtype=jnp.bfloat16)
    def randint(self, lo, hi, shape):
        return jax.random.randint(self._next(), shape, lo, hi, dtype=jnp.int32)
    def uniform(self, shape, lo=0.0, hi=1.0):
        return jax.random.uniform(self._next(), shape, jnp.bfloat16, lo, hi)
    def permutation(self, n):
        return jax.random.permutation(self._next(), n)


kernel_name = 'gated_mix__mha_block__dense_activation_mish__prompt'

def setup_inputs():
    _rng = _Rng(jax.random.key(int.from_bytes(__import__("os").urandom(4), "little")))
    _w = (lambda a: (lambda t: t.astype(jnp.bfloat16) if jnp.issubdtype(t.dtype, jnp.floating) else t)(jnp.asarray(a)))
    def _A_setup():
        B, S, D, H = 1, 2048, 640, 32
        return {
            "x": _w((lambda *s: _rng.normal(s) * 0.05)(B, S, D)),
            "wqkv": _w((lambda *s: _rng.normal(s) * 0.2)(D, 3 * D)),
            "wo": _w((lambda *s: _rng.normal(s) * 0.05)(D, D)),
        }
    _A_in = _A_setup()

    def _B_setup():
        B, S, D, F = 1, 2048, 640, 1536
        return {
            "x": _w((lambda *s: _rng.normal(s) * 0.05)(B, S, D)),
            "w1": _w((lambda *s: _rng.normal(s) * 0.8)(D, F) * (D ** -0.5)),
            "b1": _w((lambda *s: _rng.normal(s) * 0.05)(F)),
            "w2": _w((lambda *s: _rng.normal(s) * 0.05)(F, D) * (F ** -0.5)),
        }
    _B_in = _B_setup()

    return {
        "A_x": _A_in["x"],
        "A_wqkv": _A_in["wqkv"],
        "A_wo": _A_in["wo"],
        "B_x": _B_in["x"],
        "B_w1": _B_in["w1"],
        "B_b1": _B_in["b1"],
        "B_w2": _B_in["w2"],
        "gate_w": _w((lambda *s: _rng.normal(s) * 0.05)(640) * 16.0),
    }

def reference(A_x, A_wqkv, A_wo, B_x, B_w1, B_b1, B_w2, gate_w):
    def _A_ref(x, wqkv, wo):
        B, S, D = x.shape
        H = 32
        Dh = D // H
        qkv = (lambda x, *d: x.transpose(*d))((x @ wqkv).reshape(B, S, 3, H, Dh), 2, 0, 3, 1, 4)
        q, k, v = qkv[0], qkv[1], qkv[2]
        scores = jnp.einsum("bhqd,bhkd->bhqk", q, k) * (Dh ** -0.5)
        p = _softmax(scores, axis=-1)
        o = jnp.einsum("bhqk,bhkd->bhqd", p, v)
        return (lambda x, *d: x.transpose(*d))(o, 0, 2, 1, 3).reshape(B, S, D) @ wo

    def _B_ref(x, w1, b1, w2):
        h = jnp.einsum("bsd,df->bsf", x, w1) + b1
        sp = jnp.log1p(jnp.exp(-jnp.abs(h))) + jnp.where(h > 0, h, jnp.zeros_like(h))
        act = h * jnp.tanh(sp)
        return jnp.einsum("bsf,fd->bsd", act, w2)

    x = A_x
    g = _sigmoid((x * gate_w).sum(-1, keepdims=True))
    a = _A_ref(x, A_wqkv, A_wo)
    b = _B_ref(x, B_w1, B_b1, B_w2)
    return g * a + (1 - g) * b
```

```python
import jax
import jax.numpy as jnp
from jax import lax
import jax.experimental.pallas as pl
import jax.experimental.pallas.tpu as pltpu

S = 2048
D = 640
H = 32
DH = 20
F = 1536
RC = 512
NRC = S // RC
QW = 1024
NQ = 2
KT = 128
LOG2E = 1.4426950408889634
QSCALE = (DH ** -0.5) * LOG2E


def _kernel(x_hbm, wqkv_hbm, wo_hbm, w1_hbm, b1_hbm, w2_hbm, gw_hbm, o_hbm,
            x_v, wq_v, wk_v, wv_v, wo_v, w1_v, b1_v, w2_v, gw_v,
            wT_v, k_v, qT_v, vT_v, oT_v, out_v, sems):
    f32, bf16 = jnp.float32, jnp.bfloat16

    def x_copy(c):
        return pltpu.make_async_copy(x_hbm.at[pl.ds(c * RC, RC), :],
                                     x_v.at[pl.ds(c * RC, RC), :], sems.at[c])
    cp_wq = pltpu.make_async_copy(wqkv_hbm.at[:, pl.ds(0, D)], wq_v, sems.at[4])
    cp_wk = pltpu.make_async_copy(wqkv_hbm.at[:, pl.ds(D, D)], wk_v, sems.at[5])
    cp_wv = pltpu.make_async_copy(wqkv_hbm.at[:, pl.ds(2 * D, D)], wv_v, sems.at[6])
    cp_wo = pltpu.make_async_copy(wo_hbm, wo_v, sems.at[7])
    cp_w1 = pltpu.make_async_copy(w1_hbm, w1_v, sems.at[8])
    cp_b1 = pltpu.make_async_copy(b1_hbm, b1_v, sems.at[9])
    cp_w2 = pltpu.make_async_copy(w2_hbm, w2_v, sems.at[10])
    cp_gw = pltpu.make_async_copy(gw_hbm, gw_v, sems.at[11])

    cp_wk.start()
    x_copy(0).start()
    cp_wq.start()
    cp_wv.start()
    for c in range(1, NRC):
        x_copy(c).start()
    cp_wo.start()
    cp_w1.start()
    cp_b1.start()
    cp_w2.start()
    cp_gw.start()

    cp_wk.wait()
    lane = lax.broadcasted_iota(jnp.int32, (RC, 128), 1)
    for c in range(NRC):
        rows = pl.ds(c * RC, RC)
        x_copy(c).wait()
        xc = x_v[rows, :]
        kk = jnp.dot(xc, wk_v[...], preferred_element_type=f32).astype(bf16)
        kb = [kk[:, 128 * b:128 * (b + 1)] for b in range(5)]
        for b in range(5):
            k_v[b, rows, :] = kb[b]
        for b in range(4):
            off = ((128 * (b + 1)) // DH * DH) % 128
            k_v[5 + b, rows, :] = jnp.where(lane >= off, kb[b], kb[b + 1])
        if c == 0:
            cp_wq.wait()
            cp_wv.wait()
            wT_v[0:D, :] = wq_v[...].T
            wT_v[D:2 * D, :] = wv_v[...].T
        qv = lax.dot_general(wT_v[...], xc, (((1,), (1,)), ((), ())),
                             preferred_element_type=f32)
        qT_v[:, rows] = (qv[0:D, :] * QSCALE).astype(bf16)
        vT_v[:, rows] = qv[D:2 * D, :].astype(bf16).astype(f32)

    oT_v[...] = jnp.zeros(oT_v.shape, f32)
    n_qi = S // (QW * NQ)

    def head_body(i, carry):
        h = i // n_qi
        qi = i % n_qi
        start = h * DH
        blk = start // 128
        off = start % 128
        blk2 = jnp.minimum(blk + 1, 4)
        kblk = jnp.where(off > 128 - DH, blk + 5, blk)
        a8 = pl.multiple_of(start // 8 * 8, 8)
        o8 = start % 8
        r128 = lax.broadcasted_iota(jnp.int32, (128, QW), 0)
        in_head = ((r128 - off) & 127) < DH
        from_lo = r128 >= off
        r24 = lax.broadcasted_iota(jnp.int32, (24, KT), 0)
        v_valid = (r24 >= o8) & (r24 < o8 + DH)
        r24q = lax.broadcasted_iota(jnp.int32, (24, QW), 0)
        o_valid = (r24q >= o8) & (r24q < o8 + DH)

        n_kt = S // KT
        units = [(q, kt) for q in range(NQ) for kt in range(n_kt)]
        qts, accs, ms = {}, {}, {}

        def cols(q):
            return pl.ds(pl.multiple_of((qi * NQ + q) * QW, QW), QW)

        def qk(u):
            q, kt = u
            if q not in qts:
                lo = qT_v[pl.ds(pl.multiple_of(blk * 128, 128), 128), cols(q)]
                hi = qT_v[pl.ds(pl.multiple_of(blk2 * 128, 128), 128), cols(q)]
                qt = jnp.where(from_lo, lo, hi)
                qts[q] = jnp.where(in_head, qt, jnp.zeros_like(qt))
            kk = k_v[kblk, pl.ds(kt * KT, KT), :]
            return jnp.dot(kk, qts[q], preferred_element_type=f32)

        def pv(u, s):
            q, kt = u
            vt = jnp.where(v_valid, vT_v[pl.ds(a8, 24), pl.ds(kt * KT, KT)], 1.0)
            mc = jnp.max(s, axis=0, keepdims=True)
            m = mc if kt == 0 else jnp.maximum(ms[q], mc)
            p = jnp.exp2(s - m).astype(bf16)
            r = lax.dot_general(vt, p, (((1,), (0,)), ((), ())),
                                preferred_element_type=f32)
            accs[q] = r if kt == 0 else accs[q] * jnp.exp2(ms[q] - m) + r
            ms[q] = m
            if kt == n_kt - 1:
                acc = accs[q]
                l = jnp.max(jnp.where(o_valid, 0.0, acc), axis=0, keepdims=True)
                old = oT_v[pl.ds(a8, 24), cols(q)]
                oT_v[pl.ds(a8, 24), cols(q)] = jnp.where(o_valid, acc / l, old)

        s_prev = qk(units[0])
        for j in range(len(units)):
            s_next = qk(units[j + 1]) if j + 1 < len(units) else None
            pv(units[j], s_prev)
            s_prev = s_next
        return carry

    lax.fori_loop(0, H * n_qi, head_body, 0)

    cp_wo.wait()
    cp_w1.wait()
    cp_b1.wait()
    cp_w2.wait()
    cp_gw.wait()
    b1 = b1_v[...].astype(f32)
    gw = gw_v[...].astype(f32)

    def out_copy(c):
        return pltpu.make_async_copy(out_v.at[pl.ds(c * RC, RC), :],
                                     o_hbm.at[pl.ds(c * RC, RC), :], sems.at[12 + c])

    for c in range(NRC):
        rows = pl.ds(c * RC, RC)
        xc = x_v[rows, :]
        o = oT_v[:, rows].astype(bf16).T
        a = jnp.dot(o, wo_v[...], preferred_element_type=f32)
        hh = jnp.dot(xc, w1_v[...], preferred_element_type=f32) + b1
        e = jnp.exp(jnp.minimum(hh, 20.0))
        n = e * (e + 2.0)
        act = (hh * (n / (n + 2.0))).astype(bf16)
        bb = jnp.dot(act, w2_v[...], preferred_element_type=f32)
        z = jnp.sum(xc.astype(f32) * gw, axis=-1, keepdims=True)
        g = 1.0 / (1.0 + jnp.exp(-z))
        out_v[rows, :] = (g * a + (1.0 - g) * bb).astype(bf16)
        out_copy(c).start()
    for c in range(NRC):
        out_copy(c).wait()


@jax.jit
def pallas_gated_mix__mha_block__dense_activation_mish__prompt_kernel(
    A_x: jax.Array,
    A_wqkv: jax.Array,
    A_wo: jax.Array,
    B_x: jax.Array,
    B_w1: jax.Array,
    B_b1: jax.Array,
    B_w2: jax.Array,
    gate_w: jax.Array,
):
    del B_x
    f32, bf16 = jnp.float32, jnp.bfloat16
    x = A_x.reshape(S, D)
    any_spec = pl.BlockSpec(memory_space=pl.ANY)
    out = pl.pallas_call(
        _kernel,
        out_shape=jax.ShapeDtypeStruct((S, D), bf16),
        in_specs=[any_spec] * 7,
        out_specs=any_spec,
        scratch_shapes=[
            pltpu.VMEM((S, D), bf16),
            pltpu.VMEM((D, D), bf16),
            pltpu.VMEM((D, D), bf16),
            pltpu.VMEM((D, D), bf16),
            pltpu.VMEM((D, D), bf16),
            pltpu.VMEM((D, F), bf16),
            pltpu.VMEM((1, F), bf16),
            pltpu.VMEM((F, D), bf16),
            pltpu.VMEM((1, D), bf16),
            pltpu.VMEM((2 * D, D), bf16),
            pltpu.VMEM((9, S, 128), bf16),
            pltpu.VMEM((D, S), bf16),
            pltpu.VMEM((D, S), f32),
            pltpu.VMEM((D, S), f32),
            pltpu.VMEM((S, D), bf16),
            pltpu.SemaphoreType.DMA((16,)),
        ],
        compiler_params=pltpu.CompilerParams(vmem_limit_bytes=100 * 1024 * 1024),
    )(x, A_wqkv, A_wo, B_w1, B_b1.reshape(1, F), B_w2, gate_w.reshape(1, D))
    return out.reshape(1, S, D)
```

```python
import functools

import jax
import jax.numpy as jnp
from jax import lax
import jax.experimental.pallas as pl
import jax.experimental.pallas.tpu as pltpu

S = 2048
D = 640
H = 32
DH = 20
F = 1536
RC = 512
NRC = S // RC
QW = 1024
HPB = 2
KT = 128
LOG2E = 1.4426950408889634
QSCALE = (DH ** -0.5) * LOG2E
SCORE_BOUND = 56.0


def _kernel(x_hbm, wqkv_hbm, wo_hbm, w1_hbm, b1_hbm, w2_hbm, gw_hbm, o_hbm,
            x_v, wq_v, wk_v, wv_v, wo_v, w1_v, b1_v, w2_v, gw_v,
            wT_v, k_v, qm_v, vT_v, oT_v, out_v, sems):
    f32, bf16, u32 = jnp.float32, jnp.bfloat16, jnp.uint32

    def x_copy(c):
        return pltpu.make_async_copy(x_hbm.at[pl.ds(c * RC, RC), :],
                                     x_v.at[pl.ds(c * RC, RC), :], sems.at[c])
    cp_wq = pltpu.make_async_copy(wqkv_hbm.at[:, pl.ds(0, D)], wq_v, sems.at[4])
    cp_wk = pltpu.make_async_copy(wqkv_hbm.at[:, pl.ds(D, D)], wk_v, sems.at[5])
    cp_wv = pltpu.make_async_copy(wqkv_hbm.at[:, pl.ds(2 * D, D)], wv_v, sems.at[6])
    cp_wo = pltpu.make_async_copy(wo_hbm, wo_v, sems.at[7])
    cp_w1 = pltpu.make_async_copy(w1_hbm, w1_v, sems.at[8])
    cp_b1 = pltpu.make_async_copy(b1_hbm, b1_v, sems.at[9])
    cp_w2 = pltpu.make_async_copy(w2_hbm, w2_v, sems.at[10])
    cp_gw = pltpu.make_async_copy(gw_hbm, gw_v, sems.at[11])

    cp_wk.start()
    x_copy(0).start()
    x_copy(1).start()

    qm_v[...] = jnp.zeros(qm_v.shape, u32)
    lane = lax.broadcasted_iota(jnp.int32, (RC // 2, 128), 1)
    w16 = lax.broadcasted_iota(jnp.int32, (16, RC), 0)
    zero16 = jnp.zeros((16, RC), u32)

    amax = {"q": [], "k": [], "v": []}

    def track(name, t):
        t = jnp.abs(t)
        t = jnp.max(t.reshape(t.shape[0] // 8, 8, t.shape[1]), axis=0)
        amax[name].append(functools.reduce(
            jnp.maximum, [t[:, 128 * j:128 * (j + 1)] for j in range(t.shape[1] // 128)]))

    def k_proj(c):
        xc = x_v[pl.ds(c * RC, RC), :]
        kk = jnp.dot(xc, wk_v[...], preferred_element_type=f32)
        track("k", kk)
        kk = kk.astype(bf16)
        kk = pltpu.bitcast(kk, u32)
        kb = [kk[:, 128 * b:128 * (b + 1)] for b in range(5)]
        rows2 = pl.ds(c * RC // 2, RC // 2)
        for b in range(5):
            k_v[b, rows2, :] = kb[b]
        for b in range(4):
            off = ((128 * (b + 1)) // DH * DH) % 128
            k_v[5 + b, rows2, :] = jnp.where(lane >= off, kb[b], kb[b + 1])

    def qv_proj(c):
        rows = pl.ds(c * RC, RC)
        qv = lax.dot_general(wT_v[...], x_v[rows, :], (((1,), (1,)), ((), ())),
                             preferred_element_type=f32)
        qs = qv[0:D, :] * QSCALE
        track("q", qs)
        track("v", qv[D:2 * D, :])
        qt = pltpu.bitcast(qs.astype(bf16), u32)
        for h in range(H):
            w0 = (h * DH) // 16 * 8
            lo = (h * DH) // 2 - w0
            win = jnp.where((w16 >= lo) & (w16 < lo + DH // 2), qt[w0:w0 + 16, :], zero16)
            d0 = w0 % 64
            if d0 + 16 <= 64:
                qm_v[h, d0:d0 + 16, rows] = win
            else:
                qm_v[h, d0:d0 + 8, rows] = win[0:8]
                qm_v[h, 0:8, rows] = win[8:16]
        vT_v[:, rows] = qv[D:2 * D, :].astype(bf16).astype(f32)

    cp_wk.wait()
    x_copy(0).wait()
    x_copy(1).wait()
    for cp in (cp_wq, cp_wv, x_copy(2), x_copy(3), cp_wo, cp_w1, cp_b1, cp_w2, cp_gw):
        cp.start()
    k_proj(0)
    k_proj(1)
    for cp in (cp_wq, cp_wv, x_copy(2), x_copy(3)):
        cp.wait()
    wT_v[0:D, :] = wq_v[...].T
    wT_v[D:2 * D, :] = wv_v[...].T
    k_proj(2)
    k_proj(3)
    for c in range(NRC):
        qv_proj(c)
    for cp in (cp_wo, cp_w1, cp_b1, cp_w2, cp_gw):
        cp.wait()

    n_kt = S // KT
    n_q = S // QW
    n_iter = H // HPB

    def head_params(h):
        start = h * DH
        blk = lax.shift_right_logical(start, 7)
        kblk = jnp.where((start & 127) > 128 - DH, blk + 5, blk)
        return kblk, start & ~7

    def scores(h, kblk, cols, kt):
        kk = pltpu.bitcast(k_v[kblk, pl.ds(kt * (KT // 2), KT // 2), :], bf16)
        qt = pltpu.bitcast(qm_v[h, :, cols], bf16)
        return jnp.dot(kk, qt, preferred_element_type=f32)

    def pv(p, a8, o8, kt):
        r24 = lax.broadcasted_iota(jnp.int32, (24, KT), 0)
        vt = vT_v[pl.ds(pl.multiple_of(a8, 8), 24), pl.ds(kt * KT, KT)]
        vt = jnp.where((r24 >= o8) & (r24 < o8 + DH), vt, 1.0)
        return lax.dot_general(vt, p, (((1,), (0,)), ((), ())),
                               preferred_element_type=f32)

    def unshifted_body(i, carry):
        prm = [head_params(i * HPB + hh) for hh in range(HPB)]
        units = [(hh, q, kt) for hh in range(HPB) for q in range(n_q) for kt in range(n_kt)]

        def qk(u):
            hh, q, kt = u
            return scores(i * HPB + hh, prm[hh][0], pl.ds(q * QW, QW), kt)

        s_prev, acc = qk(units[0]), None
        for j, (hh, q, kt) in enumerate(units):
            s_next = qk(units[j + 1]) if j + 1 < len(units) else None
            a8, o8 = prm[hh][1], (hh * DH) % 8
            r = pv(jnp.exp2(s_prev).astype(bf16), a8, o8, kt)
            acc = r if kt == 0 else acc + r
            if kt == n_kt - 1:
                cols = pl.ds(q * QW, QW)
                lrow = 23 if o8 == 0 else 0
                o = acc * (1.0 / acc[lrow:lrow + 1, :])
                if o8 == 0:
                    oT_v[pl.ds(pl.multiple_of(a8, 8), 24), cols] = o
                else:
                    r8 = lax.broadcasted_iota(jnp.int32, (8, QW), 0)
                    first = pl.ds(pl.multiple_of(a8, 8), 8)
                    oT_v[first, cols] = jnp.where(r8 >= o8, o[0:8], oT_v[first, cols])
                    oT_v[pl.ds(pl.multiple_of(a8 + 8, 8), 16), cols] = o[8:24]
            s_prev = s_next
        return carry

    def online_body(j, carry):
        h = lax.shift_right_logical(j, 1)
        cols = pl.ds(pl.multiple_of((j & 1) * QW, QW), QW)
        kblk, a8 = head_params(h)
        o8 = (h * DH) & 7
        s_prev, acc, m = scores(h, kblk, cols, 0), None, None
        for kt in range(n_kt):
            s_next = scores(h, kblk, cols, kt + 1) if kt + 1 < n_kt else None
            mc = jnp.max(s_prev, axis=0, keepdims=True)
            m_new = mc if kt == 0 else jnp.maximum(m, mc)
            r = pv(jnp.exp2(s_prev - m_new).astype(bf16), a8, o8, kt)
            acc = r if kt == 0 else acc * jnp.exp2(m - m_new) + r
            m, s_prev = m_new, s_next
        r24 = lax.broadcasted_iota(jnp.int32, (24, QW), 0)
        valid = (r24 >= o8) & (r24 < o8 + DH)
        l = jnp.max(jnp.where(valid, 0.0, acc), axis=0, keepdims=True)
        rows = pl.ds(pl.multiple_of(a8, 8), 24)
        oT_v[rows, cols] = jnp.where(r24 >= o8, acc * (1.0 / l), oT_v[rows, cols])
        return carry

    qmax, kmax, vmax = (jnp.max(functools.reduce(jnp.maximum, amax[n])) for n in "qkv")
    safe = (DH * qmax * kmax <= SCORE_BOUND) & (vmax <= 2.0 ** 40) & (vmax >= 2.0 ** -40)

    @pl.when(safe)
    def _():
        lax.fori_loop(0, n_iter, unshifted_body, 0)

    @pl.when(jnp.logical_not(safe))
    def _():
        lax.fori_loop(0, H * n_q, online_body, 0)

    b1 = b1_v[...].astype(f32).reshape(1, F)
    gw = gw_v[...].astype(f32).reshape(1, D)

    def out_copy(c):
        return pltpu.make_async_copy(out_v.at[pl.ds(c * RC, RC), :],
                                     o_hbm.at[pl.ds(c * RC, RC), :], sems.at[12 + c])

    for c in range(NRC):
        rows = pl.ds(c * RC, RC)
        xc = x_v[rows, :]
        hh = jnp.dot(xc, w1_v[...], preferred_element_type=f32) + b1
        o = oT_v[:, rows].astype(bf16).T
        a = jnp.dot(o, wo_v[...], preferred_element_type=f32)
        e = jnp.exp(jnp.minimum(hh, 20.0))
        n = e * (e + 2.0)
        act = (hh * (n / (n + 2.0))).astype(bf16)
        bb = jnp.dot(act, w2_v[...], preferred_element_type=f32)
        z = jnp.sum(xc.astype(f32) * gw, axis=-1, keepdims=True)
        g = 1.0 / (1.0 + jnp.exp(-z))
        out_v[rows, :] = (g * a + (1.0 - g) * bb).astype(bf16)
        out_copy(c).start()
    for c in range(NRC):
        out_copy(c).wait()


@jax.jit
def pallas_gated_mix__mha_block__dense_activation_mish__prompt_kernel(
    A_x: jax.Array,
    A_wqkv: jax.Array,
    A_wo: jax.Array,
    B_x: jax.Array,
    B_w1: jax.Array,
    B_b1: jax.Array,
    B_w2: jax.Array,
    gate_w: jax.Array,
):
    del B_x
    f32, bf16 = jnp.float32, jnp.bfloat16
    x = A_x.reshape(S, D)
    any_spec = pl.BlockSpec(memory_space=pl.ANY)
    out = pl.pallas_call(
        _kernel,
        out_shape=jax.ShapeDtypeStruct((S, D), bf16),
        in_specs=[any_spec] * 7,
        out_specs=any_spec,
        scratch_shapes=[
            pltpu.VMEM((S, D), bf16),
            pltpu.VMEM((D, D), bf16),
            pltpu.VMEM((D, D), bf16),
            pltpu.VMEM((D, D), bf16),
            pltpu.VMEM((D, D), bf16),
            pltpu.VMEM((D, F), bf16),
            pltpu.VMEM((F,), bf16),
            pltpu.VMEM((F, D), bf16),
            pltpu.VMEM((D,), bf16),
            pltpu.VMEM((2 * D, D), bf16),
            pltpu.VMEM((9, S // 2, 128), jnp.uint32),
            pltpu.VMEM((H, 64, S), jnp.uint32),
            pltpu.VMEM((D, S), f32),
            pltpu.VMEM((D, S), f32),
            pltpu.VMEM((S, D), bf16),
            pltpu.SemaphoreType.DMA((16,)),
        ],
        compiler_params=pltpu.CompilerParams(vmem_limit_bytes=100 * 1024 * 1024),
    )(x, A_wqkv, A_wo, B_w1, B_b1, B_w2, gate_w)
    return out.reshape(1, S, D)
```

```python
import functools

import jax
import jax.numpy as jnp
from jax import lax
import jax.experimental.pallas as pl
import jax.experimental.pallas.tpu as pltpu

S = 2048
D = 640
H = 32
DH = 20
F = 1536
RC = 512
NRC = S // RC
OUT_CHUNKS = (768, 768, 384, 128)
QW = 1024
HPB = 2
KT = 128
LOG2E = 1.4426950408889634
QSCALE = (DH ** -0.5) * LOG2E
SCORE_BOUND = 56.0


def _kernel(x_hbm, wqkv_hbm, wo_hbm, w1_hbm, b1_hbm, w2_hbm, gw_hbm, o_hbm,
            x_v, wq_v, wk_v, wv_v, wo_v, w1_v, b1_v, w2_v, gw_v,
            wT_v, k_v, qm_v, vT_v, oT_v, pd_v, accd_v, out_v, sems):
    f32, bf16, u32 = jnp.float32, jnp.bfloat16, jnp.uint32

    def x_copy(c):
        return pltpu.make_async_copy(x_hbm.at[pl.ds(c * RC, RC), :],
                                     x_v.at[pl.ds(c * RC, RC), :], sems.at[c])
    cp_wq = pltpu.make_async_copy(wqkv_hbm.at[:, pl.ds(0, D)], wq_v, sems.at[4])
    cp_wk = pltpu.make_async_copy(wqkv_hbm.at[:, pl.ds(D, D)], wk_v, sems.at[5])
    cp_wv = pltpu.make_async_copy(wqkv_hbm.at[:, pl.ds(2 * D, D)], wv_v, sems.at[6])
    cp_wo = pltpu.make_async_copy(wo_hbm, wo_v, sems.at[7])
    cp_w1 = pltpu.make_async_copy(w1_hbm, w1_v, sems.at[8])
    cp_b1 = pltpu.make_async_copy(b1_hbm, b1_v, sems.at[9])
    cp_w2 = pltpu.make_async_copy(w2_hbm, w2_v, sems.at[10])
    cp_gw = pltpu.make_async_copy(gw_hbm, gw_v, sems.at[11])

    cp_wk.start()
    x_copy(0).start()

    qm_v[...] = jnp.zeros(qm_v.shape, u32)
    pd_v[...] = jnp.zeros(pd_v.shape, u32)
    accd_v[...] = jnp.ones(accd_v.shape, f32)
    vT_v[D:D + 24, S - KT:S] = jnp.zeros((24, KT), f32)
    oT_v[D:D + 8, S - QW:S] = jnp.zeros((8, QW), f32)
    lane = lax.broadcasted_iota(jnp.int32, (RC // 2, 128), 1)
    w16 = lax.broadcasted_iota(jnp.int32, (16, RC), 0)
    zero16 = jnp.zeros((16, RC), u32)

    amax = {"q": [], "k": [], "v": []}

    def track(name, t):
        t = jnp.abs(t)
        t = jnp.max(t.reshape(t.shape[0] // 8, 8, t.shape[1]), axis=0)
        amax[name].append(functools.reduce(
            jnp.maximum, [t[:, 128 * j:128 * (j + 1)] for j in range(t.shape[1] // 128)]))

    def k_proj(c):
        xc = x_v[pl.ds(c * RC, RC), :]
        kk = jnp.dot(xc, wk_v[...], preferred_element_type=f32)
        track("k", kk)
        kk = kk.astype(bf16)
        kk = pltpu.bitcast(kk, u32)
        kb = [kk[:, 128 * b:128 * (b + 1)] for b in range(5)]
        rows2 = pl.ds(c * RC // 2, RC // 2)
        for b in range(5):
            k_v[b, rows2, :] = kb[b]
        for b in range(4):
            off = ((128 * (b + 1)) // DH * DH) % 128
            k_v[5 + b, rows2, :] = jnp.where(lane >= off, kb[b], kb[b + 1])

    def proj_t(w_rows, c):
        return lax.dot_general(wT_v[w_rows, :], x_v[pl.ds(c * RC, RC), :],
                               (((1,), (1,)), ((), ())), preferred_element_type=f32)

    def store_v(v, c):
        track("v", v)
        vT_v[0:D, pl.ds(c * RC, RC)] = v.astype(bf16).astype(f32)

    def store_q(q, c):
        rows = pl.ds(c * RC, RC)
        qs = q * QSCALE
        track("q", qs)
        qt = pltpu.bitcast(qs.astype(bf16), u32)
        for h in range(H):
            w0 = (h * DH) // 16 * 8
            lo = (h * DH) // 2 - w0
            win = jnp.where((w16 >= lo) & (w16 < lo + DH // 2), qt[w0:w0 + 16, :], zero16)
            d0 = w0 % 64
            if d0 + 16 <= 64:
                qm_v[h, d0:d0 + 16, rows] = win
            else:
                qm_v[h, d0:d0 + 8, rows] = win[0:8]
                qm_v[h, 0:8, rows] = win[8:16]

    def qv_proj(c):
        qv = proj_t(pl.ds(0, 2 * D), c)
        store_q(qv[0:D], c)
        store_v(qv[D:2 * D], c)

    cp_wk.wait()
    x_copy(0).wait()
    for cp in (cp_wq, cp_wv, x_copy(1), x_copy(2), x_copy(3), cp_wo, cp_w1, cp_b1, cp_w2, cp_gw):
        cp.start()
    k_proj(0)
    cp_wq.wait()
    wT_v[0:D, :] = wq_v[...].T
    store_q(proj_t(pl.ds(0, D), 0), 0)
    cp_wv.wait()
    x_copy(1).wait()
    wT_v[D:2 * D, :] = wv_v[...].T
    k_proj(1)
    store_v(proj_t(pl.ds(D, D), 0), 0)
    qv_proj(1)
    x_copy(2).wait()
    x_copy(3).wait()
    for c in (2, 3):
        k_proj(c)
        qv_proj(c)
    for cp in (cp_wo, cp_w1, cp_b1, cp_w2, cp_gw):
        cp.wait()

    n_kt = S // KT
    n_q = S // QW
    n_iter = H // HPB

    def head_params(h):
        start = h * DH
        blk = lax.shift_right_logical(start, 7)
        kblk = jnp.where((start & 127) > 128 - DH, blk + 5, blk)
        return kblk, start & ~7

    def scores(h, kblk, cols, kt):
        kk = pltpu.bitcast(k_v[kblk, pl.ds(kt * (KT // 2), KT // 2), :], bf16)
        qt = pltpu.bitcast(qm_v[h, :, cols], bf16)
        return jnp.dot(kk, qt, preferred_element_type=f32)

    def pv(p, a8, o8, kt):
        r24 = lax.broadcasted_iota(jnp.int32, (24, KT), 0)
        vt = vT_v[pl.ds(pl.multiple_of(a8, 8), 24), pl.ds(kt * KT, KT)]
        vt = jnp.where((r24 >= o8) & (r24 < o8 + DH), vt, 1.0)
        return lax.dot_general(vt, p, (((1,), (0,)), ((), ())),
                               preferred_element_type=f32)

    def finish_group(acc, a8, o8, cols):
        lrow = 23 if o8 == 0 else 0
        o = acc * (1.0 / acc[lrow:lrow + 1, :])
        if o8 == 0:
            oT_v[pl.ds(pl.multiple_of(a8, 8), 24), cols] = o
        else:
            r8 = lax.broadcasted_iota(jnp.int32, (8, QW), 0)
            first = pl.ds(pl.multiple_of(a8, 8), 8)
            oT_v[first, cols] = jnp.where(r8 >= o8, o[0:8], oT_v[first, cols])
            oT_v[pl.ds(pl.multiple_of(a8 + 8, 8), 16), cols] = o[8:24]

    def finish_deferred(a8):
        o8 = ((HPB - 1) * DH) % 8
        r = pv(pltpu.bitcast(pd_v[...], bf16), a8, o8, n_kt - 1)
        finish_group(accd_v[...] + r, a8, o8, pl.ds(S - QW, QW))

    def unshifted_body(i, carry):
        prm = [head_params(i * HPB + hh) for hh in range(HPB)]
        units = [(hh, q, kt) for hh in range(HPB) for q in range(n_q) for kt in range(n_kt)]

        def qk(u):
            hh, q, kt = u
            return scores(i * HPB + hh, prm[hh][0], pl.ds(q * QW, QW), kt)

        s_prev, acc = qk(units[0]), None
        finish_deferred(jnp.where(i == 0, D, ((i * HPB - 1) * DH) & ~7))
        for j, (hh, q, kt) in enumerate(units):
            p = jnp.exp2(s_prev).astype(bf16)
            if j + 1 == len(units):
                pd_v[...] = pltpu.bitcast(p, u32)
                accd_v[...] = acc
                break
            s_prev = qk(units[j + 1])
            a8, o8 = prm[hh][1], (hh * DH) % 8
            r = pv(p, a8, o8, kt)
            acc = r if kt == 0 else acc + r
            if kt == n_kt - 1:
                finish_group(acc, a8, o8, pl.ds(q * QW, QW))
        return carry

    def online_body(j, carry):
        h = lax.shift_right_logical(j, 1)
        cols = pl.ds(pl.multiple_of((j & 1) * QW, QW), QW)
        kblk, a8 = head_params(h)
        o8 = (h * DH) & 7
        s_prev, acc, m = scores(h, kblk, cols, 0), None, None
        for kt in range(n_kt):
            s_next = scores(h, kblk, cols, kt + 1) if kt + 1 < n_kt else None
            mc = jnp.max(s_prev, axis=0, keepdims=True)
            m_new = mc if kt == 0 else jnp.maximum(m, mc)
            r = pv(jnp.exp2(s_prev - m_new).astype(bf16), a8, o8, kt)
            acc = r if kt == 0 else acc * jnp.exp2(m - m_new) + r
            m, s_prev = m_new, s_next
        r24 = lax.broadcasted_iota(jnp.int32, (24, QW), 0)
        valid = (r24 >= o8) & (r24 < o8 + DH)
        l = jnp.max(jnp.where(valid, 0.0, acc), axis=0, keepdims=True)
        rows = pl.ds(pl.multiple_of(a8, 8), 24)
        oT_v[rows, cols] = jnp.where(r24 >= o8, acc * (1.0 / l), oT_v[rows, cols])
        return carry

    qmax, kmax, vmax = (jnp.max(functools.reduce(jnp.maximum, amax[n])) for n in "qkv")
    safe = (DH * qmax * kmax <= SCORE_BOUND) & (vmax <= 2.0 ** 40) & (vmax >= 2.0 ** -40)

    @pl.when(safe)
    def _():
        lax.fori_loop(0, n_iter, unshifted_body, 0)
        finish_deferred(((H - 1) * DH) & ~7)

    @pl.when(jnp.logical_not(safe))
    def _():
        lax.fori_loop(0, H * n_q, online_body, 0)

    b1 = b1_v[...].astype(f32).reshape(1, F)
    gw = gw_v[...].astype(f32).reshape(1, D)

    def out_copy(r0, nr, k):
        return pltpu.make_async_copy(out_v.at[pl.ds(r0, nr), :],
                                     o_hbm.at[pl.ds(r0, nr), :], sems.at[12 + k])

    copies = []
    r0 = 0
    for rc in OUT_CHUNKS:
        rows = pl.ds(r0, rc)
        xc = x_v[rows, :]
        hh = jnp.dot(xc, w1_v[...], preferred_element_type=f32) + b1
        o = oT_v[0:D, rows].astype(bf16).T
        a = jnp.dot(o, wo_v[...], preferred_element_type=f32)
        e = jnp.exp(jnp.minimum(hh, 20.0))
        n = e * (e + 2.0)
        act = (hh * (n / (n + 2.0))).astype(bf16)
        z = jnp.sum(xc.astype(f32) * gw, axis=-1, keepdims=True)
        g = 1.0 / (1.0 + jnp.exp(-z))
        bb = jnp.dot(act, w2_v[...], preferred_element_type=f32)
        out_v[rows, :] = (g * a + (1.0 - g) * bb).astype(bf16)
        copies.append(out_copy(r0, rc, len(copies)))
        copies[-1].start()
        r0 += rc
    for cp in copies:
        cp.wait()


@jax.jit
def pallas_gated_mix__mha_block__dense_activation_mish__prompt_kernel(
    A_x: jax.Array,
    A_wqkv: jax.Array,
    A_wo: jax.Array,
    B_x: jax.Array,
    B_w1: jax.Array,
    B_b1: jax.Array,
    B_w2: jax.Array,
    gate_w: jax.Array,
):
    del B_x
    f32, bf16 = jnp.float32, jnp.bfloat16
    x = A_x.reshape(S, D)
    any_spec = pl.BlockSpec(memory_space=pl.ANY)
    out = pl.pallas_call(
        _kernel,
        out_shape=jax.ShapeDtypeStruct((S, D), bf16),
        in_specs=[any_spec] * 7,
        out_specs=any_spec,
        scratch_shapes=[
            pltpu.VMEM((S, D), bf16),
            pltpu.VMEM((D, D), bf16),
            pltpu.VMEM((D, D), bf16),
            pltpu.VMEM((D, D), bf16),
            pltpu.VMEM((D, D), bf16),
            pltpu.VMEM((D, F), bf16),
            pltpu.VMEM((F,), bf16),
            pltpu.VMEM((F, D), bf16),
            pltpu.VMEM((D,), bf16),
            pltpu.VMEM((2 * D, D), bf16),
            pltpu.VMEM((9, S // 2, 128), jnp.uint32),
            pltpu.VMEM((H, 64, S), jnp.uint32),
            pltpu.VMEM((D + 24, S), f32),
            pltpu.VMEM((D + 24, S), f32),
            pltpu.VMEM((KT // 2, QW), jnp.uint32),
            pltpu.VMEM((24, QW), f32),
            pltpu.VMEM((S, D), bf16),
            pltpu.SemaphoreType.DMA((12 + len(OUT_CHUNKS),)),
        ],
        compiler_params=pltpu.CompilerParams(vmem_limit_bytes=100 * 1024 * 1024),
    )(x, A_wqkv, A_wo, B_w1, B_b1, B_w2, gate_w)
    return out.reshape(1, S, D)
```
